```python
import jax
import jax.numpy as jnp

def _softmax(x, axis=-1):
    return jax.nn.softmax(x, axis=axis)
def _gelu(x):
    return jax.nn.gelu(x, approximate=True)
def _silu(x):
    return jax.nn.silu(x)
def _sigmoid(x):
    return jax.nn.sigmoid(x)
def _layernorm(x, axis=-1, eps=1e-5):
    m = jnp.mean(x, axis=axis, keepdims=True)
    v = jnp.var(x, axis=axis, keepdims=True)
    return (x - m) / jnp.sqrt(v + eps)
def _scatter_add(tgt, idx, src, axis=0):
    return tgt.at[idx].add(src)
def _segment_sum(src, seg, n):
    return jax.ops.segment_sum(src, seg, n)
class _Rng:
    def __init__(self, key):
        self._k = key
    def _next(self):
        self._k, sub = jax.random.split(self._k)
        return sub
    def normal(self, shape):
        return jax.random.normal(self._next(), shape, dtype=jnp.bfloat16)
    def randint(self, lo, hi, shape):
        return jax.random.randint(self._next(), shape, lo, hi, dtype=jnp.int32)
    def uniform(self, shape, lo=0.0, hi=1.0):
        return jax.random.uniform(self._next(), shape, jnp.bfloat16, lo, hi)
    def permutation(self, n):
        return jax.random.permutation(self._next(), n)


kernel_name = 'recurrent_scan__sliding_block_cached__moe_arch_mod__decode'

def setup_inputs():
    _rng = _Rng(jax.random.key(int.from_bytes(__import__("os").urandom(4), "little")))
    _w = (lambda a: (lambda t: t.astype(jnp.bfloat16) if jnp.issubdtype(t.dtype, jnp.floating) else t)(jnp.asarray(a)))
    def _A_setup():
        B, Sq, D = 1, 1, 512
        Hq, Hkv, Sk, Dh = 32, 32, 32768, 128
        assert Hq % Hkv == 0, (Hq, Hkv)
        return {
            "x": _w((lambda *s: _rng.normal(s) * 0.05)(B, Sq, D)),
            "k_cache": _w((lambda *s: _rng.normal(s) * 0.05)(B, Hkv, Sk, Dh)),
            "v_cache": _w((lambda *s: _rng.normal(s) * 0.05)(B, Hkv, Sk, Dh)),
            "wq": _w((lambda *s: _rng.normal(s) * 0.05)(D, Hq * Dh) * (D ** -0.5)),
            "wo": _w((lambda *s: _rng.normal(s) * 0.05)(Hq * Dh, D) * ((Hq * Dh) ** -0.5)),
        }
    _A_in = _A_setup()

    def _B_setup():
        B, S, D, F, C = 1, 1, 512, 1376, 1
        return {
            "x": _w((lambda *s: _rng.normal(s) * 0.05)(B, S, D)),
            "w_r": _w((lambda *s: _rng.normal(s) * 0.05)(D)),
            "w_gate": _w((lambda *s: _rng.normal(s) * 0.05)(D, F)),
            "w_up": _w((lambda *s: _rng.normal(s) * 0.05)(D, F)),
            "w_down": _w((lambda *s: _rng.normal(s) * 0.05)(F, D)),
        }
    _B_in = _B_setup()

    return {
        "A_x": _A_in["x"],
        "A_k_cache": _A_in["k_cache"],
        "A_v_cache": _A_in["v_cache"],
        "A_wq": _A_in["wq"],
        "A_wo": _A_in["wo"],
        "B_x": _B_in["x"],
        "B_w_r": _B_in["w_r"],
        "B_w_gate": _B_in["w_gate"],
        "B_w_up": _B_in["w_up"],
        "B_w_down": _B_in["w_down"],
    }

def reference(A_x, A_k_cache, A_v_cache, A_wq, A_wo, B_x, B_w_r, B_w_gate, B_w_up, B_w_down):
    def _A_ref(x, k_cache, v_cache, wq, wo):
        B, Sq, D = x.shape
        Hq, Dh = 32, 128
        Hkv, Sk = k_cache.shape[1], k_cache.shape[2]
        W = min(4096, max(256, Sk // 4))
        rep = Hq // Hkv
        q = (lambda x, *d: x.transpose(*d))((x @ wq).reshape(B, Sq, Hq, Dh), 0, 2, 1, 3)
        k = jnp.repeat(k_cache[:, :, Sk - W:, :], rep, axis=1)
        v = jnp.repeat(v_cache[:, :, Sk - W:, :], rep, axis=1)
        scores = jnp.einsum("bhqd,bhkd->bhqk", q, k) * (Dh ** -0.5)
        p = _softmax(scores, axis=-1)
        o = jnp.einsum("bhqk,bhkd->bhqd", p, v)
        return (lambda x, *d: x.transpose(*d))(o, 0, 2, 1, 3).reshape(B, Sq, Hq * Dh) @ wo

    def _B_ref(x, w_r, w_gate, w_up, w_down):
        B, S, D = x.shape
        C = 1
        r = x @ w_r
        idx = jnp.argsort(-r, axis=-1)[:, :C]
        idx_e = jnp.repeat(idx.reshape(B, C, 1), D, axis=2)
        x_sel = jnp.take_along_axis(x, idx_e, axis=1)
        g = _silu(x_sel @ w_gate)
        u = x_sel @ w_up
        y = (g * u) @ w_down
        r_sel = _sigmoid(jnp.take_along_axis(r, idx, axis=1))
        y = y * r_sel.reshape(B, C, 1)
        b_off = (jnp.arange(B) * S).reshape(B, 1)
        flat_idx = (idx + b_off).reshape(B * C)
        zero = (x * 0.0).reshape(B * S, D)
        upd = _scatter_add(zero, flat_idx, y.reshape(B * C, D), axis=0)
        return x + upd.reshape(B, S, D)

    x = A_x
    xn = _layernorm(x, axis=-1)
    s = _A_ref(xn, A_k_cache, A_v_cache, A_wq, A_wo)
    g = _silu(_B_ref(xn, B_w_r, B_w_gate, B_w_up, B_w_down))
    return x + s * g
```

```python
import jax
import jax.numpy as jnp
from jax import lax
from jax.experimental import pallas as pl
from jax.experimental.pallas import tpu as pltpu

F32, BF16 = jnp.float32, jnp.bfloat16
NT = (((1,), (1,)), ((), ()))

KV_CHUNKS = (4,) * 8
WO_CHUNKS = (16, 8, 4, 2, 2)


def _offsets(chunks):
    return [sum(chunks[:i]) for i in range(len(chunks))]


@jax.jit
def pallas_recurrent_scan__sliding_block_cached__moe_arch_mod__decode_kernel(
    A_x: jax.Array,
    A_k_cache: jax.Array,
    A_v_cache: jax.Array,
    A_wq: jax.Array,
    A_wo: jax.Array,
    B_x: jax.Array,
    B_w_r: jax.Array,
    B_w_gate: jax.Array,
    B_w_up: jax.Array,
    B_w_down: jax.Array,
):
    del B_x
    _, H, SK, DH = A_k_cache.shape
    D = A_x.shape[-1]
    F = B_w_gate.shape[1]
    W = min(4096, max(256, SK // 4))
    scale = DH ** -0.5
    kv_off, wo_off = _offsets(KV_CHUNKS), _offsets(WO_CHUNKS)
    n_sems = 6 + 2 * len(KV_CHUNKS) + len(WO_CHUNKS)

    def kernel(x_hbm, k_hbm, v_hbm, wq_hbm, wo_hbm, wr_hbm, wg_hbm, wu_hbm, wd_hbm, o_ref,
               x_vm, wr_vm, wq_vm, k_vm, v_vm, wo_vm, wg_vm, wu_vm, wd_vm, q_vm, oh_vm, sems):
        sem_ids = iter(range(n_sems))

        def copy(src, dst):
            return pltpu.make_async_copy(src, dst, sems.at[next(sem_ids)])

        x_cp, wr_cp, wq_cp = copy(x_hbm, x_vm), copy(wr_hbm, wr_vm), copy(wq_hbm, wq_vm)
        wg_cp, wu_cp, wd_cp = copy(wg_hbm, wg_vm), copy(wu_hbm, wu_vm), copy(wd_hbm, wd_vm)
        k_cp, v_cp, wo_cp = [], [], []
        for o, n in zip(kv_off, KV_CHUNKS):
            k_cp.append(copy(k_hbm.at[0, pl.ds(o, n), pl.ds(SK - W, W), :], k_vm.at[pl.ds(o, n)]))
            v_cp.append(copy(v_hbm.at[0, pl.ds(o, n), pl.ds(SK - W, W), :], v_vm.at[pl.ds(o, n)]))
        for o, n in zip(wo_off, WO_CHUNKS):
            rows = pl.ds(o * DH, n * DH)
            wo_cp.append(copy(wo_hbm.at[rows, :], wo_vm.at[rows, :]))

        x_cp.start()
        wr_cp.start()
        wq_cp.start()
        for kc, vc in zip(k_cp, v_cp):
            kc.start()
            vc.start()
        wg_cp.start()
        wu_cp.start()
        wd_cp.start()
        for c in wo_cp:
            c.start()

        x_cp.wait()
        x = x_vm[0].astype(F32)
        xc = x - jnp.mean(x, axis=-1, keepdims=True)
        var = jnp.mean(xc * xc, axis=-1, keepdims=True)
        xn = (xc / jnp.sqrt(var + 1e-5)).astype(BF16)
        xn32 = xn.astype(F32)
        wr_cp.wait()
        r = jnp.sum(xn32 * wr_vm[...].reshape(1, D).astype(F32), axis=-1, keepdims=True)

        wq_cp.wait()
        q_vm[...] = jnp.dot(xn, wq_vm[...], preferred_element_type=F32).astype(BF16)

        def head(h, carry):
            lanes = pl.ds(pl.multiple_of(h * DH, DH), DH)
            s = lax.dot_general(q_vm[:, lanes], k_vm[h], NT, preferred_element_type=F32) * scale
            p = jnp.exp(s - jnp.max(s, axis=-1, keepdims=True))
            l = jnp.sum(p, axis=-1, keepdims=True)
            o = jnp.dot(p.astype(BF16), v_vm[h], preferred_element_type=F32)
            oh_vm[:, lanes] = (o / l).astype(BF16)
            return carry

        for kc, vc, o, n in zip(k_cp, v_cp, kv_off, KV_CHUNKS):
            kc.wait()
            vc.wait()
            lax.fori_loop(o, o + n, head, None)

        wg_cp.wait()
        wu_cp.wait()
        gp = lax.dot_general(xn, wg_vm[...], NT, preferred_element_type=F32).astype(BF16).astype(F32)
        up = lax.dot_general(xn, wu_vm[...], NT, preferred_element_type=F32).astype(BF16).astype(F32)
        g = (gp * jax.nn.sigmoid(gp)).astype(BF16).astype(F32)
        wd_cp.wait()
        y = jnp.dot((g * up).astype(BF16), wd_vm[...], preferred_element_type=F32)
        y = y * jax.nn.sigmoid(r)
        z = xn32 + (xn32 * 0.0 + y)
        gate = z * jax.nn.sigmoid(z)

        acc = None
        for c, o, n in zip(wo_cp, wo_off, WO_CHUNKS):
            c.wait()
            part = jnp.dot(oh_vm[:, o * DH:(o + n) * DH], wo_vm[o * DH:(o + n) * DH, :],
                           preferred_element_type=F32)
            acc = part if acc is None else acc + part
        o_ref[0] = (x + acc * gate).astype(o_ref.dtype)

    hbm = pl.BlockSpec(memory_space=pl.ANY)
    return pl.pallas_call(
        kernel,
        out_shape=jax.ShapeDtypeStruct((1, 1, D), A_x.dtype),
        in_specs=[hbm] * 9,
        out_specs=pl.BlockSpec(memory_space=pltpu.VMEM),
        scratch_shapes=[
            pltpu.VMEM((1, 1, D), BF16),
            pltpu.VMEM((D,), BF16),
            pltpu.VMEM((D, H * DH), BF16),
            pltpu.VMEM((H, W, DH), BF16),
            pltpu.VMEM((H, W, DH), BF16),
            pltpu.VMEM((H * DH, D), BF16),
            pltpu.VMEM((F, D), BF16),
            pltpu.VMEM((F, D), BF16),
            pltpu.VMEM((F, D), BF16),
            pltpu.VMEM((1, H * DH), BF16),
            pltpu.VMEM((1, H * DH), BF16),
            pltpu.SemaphoreType.DMA((n_sems,)),
        ],
        compiler_params=pltpu.CompilerParams(vmem_limit_bytes=100 * 1024 * 1024),
    )(A_x, A_k_cache, A_v_cache, A_wq, A_wo, B_w_r, B_w_gate.T, B_w_up.T, B_w_down)
```

```python
import jax
import jax.numpy as jnp
from jax import lax
from jax.experimental import pallas as pl
from jax.experimental.pallas import tpu as pltpu

F32, BF16 = jnp.float32, jnp.bfloat16
NT = (((1,), (1,)), ((), ()))

KV_HEADS = (4,) * 8
WO_MXU_ROWS = (1024, 1024, 1024, 512, 256, 128)
WO_VPU_ROWS = (96, 32)


def _offsets(sizes, start=0):
    return [start + sum(sizes[:i]) for i in range(len(sizes))]


@jax.jit
def pallas_recurrent_scan__sliding_block_cached__moe_arch_mod__decode_kernel(
    A_x: jax.Array,
    A_k_cache: jax.Array,
    A_v_cache: jax.Array,
    A_wq: jax.Array,
    A_wo: jax.Array,
    B_x: jax.Array,
    B_w_r: jax.Array,
    B_w_gate: jax.Array,
    B_w_up: jax.Array,
    B_w_down: jax.Array,
):
    del B_x
    _, H, SK, DH = A_k_cache.shape
    D = A_x.shape[-1]
    F = B_w_gate.shape[1]
    W = min(4096, max(256, SK // 4))
    scale = DH ** -0.5
    assert sum(KV_HEADS) == H and sum(WO_VPU_ROWS) == DH
    assert sum(WO_MXU_ROWS) + DH == H * DH
    vpu0 = H * DH - DH
    kv_off = _offsets(KV_HEADS)
    mxu_off, vpu_off = _offsets(WO_MXU_ROWS), _offsets(WO_VPU_ROWS, vpu0)
    n_sems = 6 + 2 * len(KV_HEADS) + len(WO_MXU_ROWS) + len(WO_VPU_ROWS)

    def kernel(x_hbm, k_hbm, v_hbm, wq_hbm, wo_hbm, wr_hbm, wg_hbm, wu_hbm, wd_hbm, o_ref,
               x_vm, wr_vm, wq_vm, k_vm, v_vm, wo_vm, wg_vm, wu_vm, wd_vm, q_vm, oh_vm):
        def body(sems):
            sem_ids = iter(range(n_sems))

            def copy(src, dst):
                return pltpu.make_async_copy(src, dst, sems.at[next(sem_ids)])

            def wo_copy(o, n):
                return copy(wo_hbm.at[pl.ds(o, n), :], wo_vm.at[pl.ds(o, n), :])

            x_cp, wr_cp, wq_cp = copy(x_hbm, x_vm), copy(wr_hbm, wr_vm), copy(wq_hbm, wq_vm)
            wg_cp, wu_cp, wd_cp = copy(wg_hbm, wg_vm), copy(wu_hbm, wu_vm), copy(wd_hbm, wd_vm)
            k_cp, v_cp = [], []
            for h0, n in zip(kv_off, KV_HEADS):
                window = (0, pl.ds(h0, n), pl.ds(SK - W, W), slice(None))
                k_cp.append(copy(k_hbm.at[window], k_vm.at[pl.ds(h0, n)]))
                v_cp.append(copy(v_hbm.at[window], v_vm.at[pl.ds(h0, n)]))
            mxu_cp = [wo_copy(o, n) for o, n in zip(mxu_off, WO_MXU_ROWS)]
            vpu_cp = [wo_copy(o, n) for o, n in zip(vpu_off, WO_VPU_ROWS)]

            wq_cp.start()
            x_cp.start()
            wr_cp.start()
            for kc, vc in zip(k_cp, v_cp):
                kc.start()
                vc.start()
            wg_cp.start()
            wu_cp.start()
            wd_cp.start()
            for c in mxu_cp + vpu_cp:
                c.start()

            x_cp.wait()
            x = x_vm[0].astype(F32)
            xc = x - jnp.mean(x, axis=-1, keepdims=True)
            var = jnp.mean(xc * xc, axis=-1, keepdims=True)
            xn = (xc / jnp.sqrt(var + 1e-5)).astype(BF16)
            xn32 = xn.astype(F32)
            wr_cp.wait()
            r = jnp.sum(xn32 * wr_vm[...].reshape(1, D).astype(F32), axis=-1, keepdims=True)

            wq_cp.wait()
            q_vm[...] = jnp.dot(xn, wq_vm[...], preferred_element_type=F32).astype(BF16)

            def head(h, carry):
                lanes = pl.ds(pl.multiple_of(h * DH, DH), DH)
                s = lax.dot_general(q_vm[:, lanes], k_vm[h], NT, preferred_element_type=F32) * scale
                p = jnp.exp(s - jnp.max(s, axis=-1, keepdims=True))
                denom = jnp.sum(p, axis=-1, keepdims=True)
                o = jnp.dot(p.astype(BF16), v_vm[h], preferred_element_type=F32)
                oh_vm[:, lanes] = (o / denom).astype(BF16)
                return carry

            for kc, vc, h0, n in zip(k_cp, v_cp, kv_off, KV_HEADS):
                kc.wait()
                vc.wait()
                lax.fori_loop(h0, h0 + n, head, None)

            wg_cp.wait()
            wu_cp.wait()
            gp = lax.dot_general(xn, wg_vm[...], NT, preferred_element_type=F32).astype(BF16).astype(F32)
            up = lax.dot_general(xn, wu_vm[...], NT, preferred_element_type=F32).astype(BF16).astype(F32)
            act = (gp * jax.nn.sigmoid(gp)).astype(BF16).astype(F32)
            wd_cp.wait()
            y = jnp.dot((act * up).astype(BF16), wd_vm[...], preferred_element_type=F32)
            y = y * jax.nn.sigmoid(r)
            z = xn32 + (xn32 * 0.0 + y)
            gate = z * jax.nn.sigmoid(z)

            eye = (lax.broadcasted_iota(jnp.int32, (DH, DH), 0)
                   == lax.broadcasted_iota(jnp.int32, (DH, DH), 1))
            o_last = jnp.broadcast_to(oh_vm[:, vpu0:].astype(F32), (DH, DH))
            o_col = jnp.sum(jnp.where(eye, o_last, 0.0), axis=1, keepdims=True)

            acc = jnp.zeros((1, D), F32)
            for c, o, n in zip(mxu_cp, mxu_off, WO_MXU_ROWS):
                c.wait()
                acc = acc + jnp.dot(oh_vm[:, o:o + n], wo_vm[o:o + n, :], preferred_element_type=F32)
            base = x + acc * gate
            acc8 = jnp.zeros((8, D), F32)
            for c, o, n in zip(vpu_cp, vpu_off, WO_VPU_ROWS):
                c.wait()
                prod = wo_vm[o:o + n, :].astype(F32) * o_col[o - vpu0:o - vpu0 + n]
                acc8 = acc8 + jnp.sum(prod.reshape(n // 8, 8, D), axis=0)
            o_ref[0] = (base + jnp.sum(acc8, axis=0, keepdims=True) * gate).astype(o_ref.dtype)

        pl.run_scoped(body, pltpu.SemaphoreType.DMA((n_sems,)))

    return pl.pallas_call(
        kernel,
        out_shape=jax.ShapeDtypeStruct((1, 1, D), A_x.dtype),
        in_specs=[pl.BlockSpec(memory_space=pl.ANY)] * 9,
        out_specs=pl.BlockSpec(memory_space=pltpu.VMEM),
        scratch_shapes=[
            pltpu.VMEM((1, 1, D), BF16),
            pltpu.VMEM((D,), BF16),
            pltpu.VMEM((D, H * DH), BF16),
            pltpu.VMEM((H, W, DH), BF16),
            pltpu.VMEM((H, W, DH), BF16),
            pltpu.VMEM((H * DH, D), BF16),
            pltpu.VMEM((F, D), BF16),
            pltpu.VMEM((F, D), BF16),
            pltpu.VMEM((F, D), BF16),
            pltpu.VMEM((1, H * DH), BF16),
            pltpu.VMEM((1, H * DH), BF16),
        ],
        compiler_params=pltpu.CompilerParams(vmem_limit_bytes=100 * 1024 * 1024),
    )(A_x, A_k_cache, A_v_cache, A_wq, A_wo, B_w_r, B_w_gate.T, B_w_up.T, B_w_down)
```

```python
import jax
import jax.numpy as jnp
from jax import lax
from jax.experimental import pallas as pl
from jax.experimental.pallas import tpu as pltpu

F32, BF16 = jnp.float32, jnp.bfloat16
NT = (((1,), (1,)), ((), ()))

KV_HEADS = (4,) * 8
WO_MXU_ROWS = (1024, 1024, 1024, 512, 256, 128)
WO_VPU_ROWS = (80, 32, 16)


def _offsets(sizes, start=0):
    return [start + sum(sizes[:i]) for i in range(len(sizes))]


@jax.jit
def pallas_recurrent_scan__sliding_block_cached__moe_arch_mod__decode_kernel(
    A_x: jax.Array,
    A_k_cache: jax.Array,
    A_v_cache: jax.Array,
    A_wq: jax.Array,
    A_wo: jax.Array,
    B_x: jax.Array,
    B_w_r: jax.Array,
    B_w_gate: jax.Array,
    B_w_up: jax.Array,
    B_w_down: jax.Array,
):
    del B_x
    _, H, SK, DH = A_k_cache.shape
    D = A_x.shape[-1]
    F = B_w_gate.shape[1]
    W = min(4096, max(256, SK // 4))
    scale = DH ** -0.5
    assert sum(KV_HEADS) == H and sum(WO_VPU_ROWS) == DH
    assert sum(WO_MXU_ROWS) + DH == H * DH
    vpu0 = H * DH - DH
    kv_off = _offsets(KV_HEADS)
    mxu_off, vpu_off = _offsets(WO_MXU_ROWS), _offsets(WO_VPU_ROWS, vpu0)
    n_sems = 6 + 2 * len(KV_HEADS) + len(WO_MXU_ROWS) + len(WO_VPU_ROWS)

    def kernel(x_hbm, k_hbm, v_hbm, wq_hbm, wo_hbm, wr_hbm, wg_hbm, wu_hbm, wd_hbm, o_ref,
               x_vm, wr_vm, wq_vm, k_vm, v_vm, wo_vm, wg_vm, wu_vm, wd_vm, q_vm, oh_vm):
        def body(sems):
            sem_ids = iter(range(n_sems))

            def copy(src, dst):
                return pltpu.make_async_copy(src, dst, sems.at[next(sem_ids)])

            def wo_copy(o, n):
                return copy(wo_hbm.at[pl.ds(o, n), :], wo_vm.at[pl.ds(o, n), :])

            x_cp, wr_cp, wq_cp = copy(x_hbm, x_vm), copy(wr_hbm, wr_vm), copy(wq_hbm, wq_vm)
            wg_cp, wu_cp, wd_cp = copy(wg_hbm, wg_vm), copy(wu_hbm, wu_vm), copy(wd_hbm, wd_vm)
            k_cp, v_cp = [], []
            for h0, n in zip(kv_off, KV_HEADS):
                window = (0, pl.ds(h0, n), pl.ds(SK - W, W), slice(None))
                k_cp.append(copy(k_hbm.at[window], k_vm.at[pl.ds(h0, n)]))
                v_cp.append(copy(v_hbm.at[window], v_vm.at[pl.ds(h0, n)]))
            mxu_cp = [wo_copy(o, n) for o, n in zip(mxu_off, WO_MXU_ROWS)]
            vpu_cp = [wo_copy(o, n) for o, n in zip(vpu_off, WO_VPU_ROWS)]

            wq_cp.start()
            x_cp.start()
            wr_cp.start()
            for kc, vc in zip(k_cp, v_cp):
                kc.start()
                vc.start()
            wg_cp.start()
            wu_cp.start()
            wd_cp.start()
            for c in mxu_cp + vpu_cp:
                c.start()

            x_cp.wait()
            x = x_vm[0].astype(F32)
            xc = x - jnp.mean(x, axis=-1, keepdims=True)
            var = jnp.mean(xc * xc, axis=-1, keepdims=True)
            xn = (xc / jnp.sqrt(var + 1e-5)).astype(BF16)
            xn32 = xn.astype(F32)
            wr_cp.wait()
            r = jnp.sum(xn32 * wr_vm[...].reshape(1, D).astype(F32), axis=-1, keepdims=True)

            wq_cp.wait()
            q_vm[...] = jnp.dot(xn, wq_vm[...], preferred_element_type=F32).astype(BF16)

            def head(h, carry):
                lanes = pl.ds(pl.multiple_of(h * DH, DH), DH)
                s = lax.dot_general(q_vm[:, lanes], k_vm[h], NT, preferred_element_type=F32) * scale
                p = jnp.exp(s - jnp.max(s, axis=-1, keepdims=True))
                denom = jnp.sum(p, axis=-1, keepdims=True)
                o = jnp.dot(p.astype(BF16), v_vm[h], preferred_element_type=F32)
                oh_vm[:, lanes] = (o / denom).astype(BF16)
                return carry

            for kc, vc, h0, n in zip(k_cp, v_cp, kv_off, KV_HEADS):
                kc.wait()
                vc.wait()
                lax.fori_loop(h0, h0 + n, head, None)

            wg_cp.wait()
            wu_cp.wait()
            gp = lax.dot_general(xn, wg_vm[...], NT, preferred_element_type=F32).astype(BF16).astype(F32)
            up = lax.dot_general(xn, wu_vm[...], NT, preferred_element_type=F32).astype(BF16).astype(F32)
            act = (gp * jax.nn.sigmoid(gp)).astype(BF16).astype(F32)
            wd_cp.wait()
            y = jnp.dot((act * up).astype(BF16), wd_vm[...], preferred_element_type=F32)
            y = y * jax.nn.sigmoid(r)
            z = xn32 + (xn32 * 0.0 + y)
            gate = z * jax.nn.sigmoid(z)

            eye = (lax.broadcasted_iota(jnp.int32, (DH, DH), 0)
                   == lax.broadcasted_iota(jnp.int32, (DH, DH), 1))
            o_last = jnp.broadcast_to(oh_vm[:, vpu0:].astype(F32), (DH, DH))
            o_col = jnp.sum(jnp.where(eye, o_last, 0.0), axis=1, keepdims=True)

            acc = jnp.zeros((1, D), F32)
            for c, o, n in zip(mxu_cp, mxu_off, WO_MXU_ROWS):
                c.wait()
                acc = acc + jnp.dot(oh_vm[:, o:o + n], wo_vm[o:o + n, :], preferred_element_type=F32)
            row0 = lax.broadcasted_iota(jnp.int32, (8, D), 0) == 0
            acc8 = jnp.where(row0, jnp.broadcast_to(x + acc * gate, (8, D)), 0.0)
            for c, o, n in zip(vpu_cp, vpu_off, WO_VPU_ROWS):
                coef = o_col[o - vpu0:o - vpu0 + n] * gate
                c.wait()
                prod = wo_vm[o:o + n, :].astype(F32) * coef
                acc8 = acc8 + jnp.sum(prod.reshape(n // 8, 8, D), axis=0)
            o_ref[0] = jnp.sum(acc8, axis=0, keepdims=True).astype(o_ref.dtype)

        pl.run_scoped(body, pltpu.SemaphoreType.DMA((n_sems,)))

    return pl.pallas_call(
        kernel,
        out_shape=jax.ShapeDtypeStruct((1, 1, D), A_x.dtype),
        in_specs=[pl.BlockSpec(memory_space=pl.ANY)] * 9,
        out_specs=pl.BlockSpec(memory_space=pltpu.VMEM),
        scratch_shapes=[
            pltpu.VMEM((1, 1, D), BF16),
            pltpu.VMEM((D,), BF16),
            pltpu.VMEM((D, H * DH), BF16),
            pltpu.VMEM((H, W, DH), BF16),
            pltpu.VMEM((H, W, DH), BF16),
            pltpu.VMEM((H * DH, D), BF16),
            pltpu.VMEM((F, D), BF16),
            pltpu.VMEM((F, D), BF16),
            pltpu.VMEM((F, D), BF16),
            pltpu.VMEM((1, H * DH), BF16),
            pltpu.VMEM((1, H * DH), BF16),
        ],
        compiler_params=pltpu.CompilerParams(vmem_limit_bytes=100 * 1024 * 1024),
    )(A_x, A_k_cache, A_v_cache, A_wq, A_wo, B_w_r, B_w_gate.T, B_w_up.T, B_w_down)
```
